```python
import jax
import jax.numpy as jnp

def _softmax(x, axis=-1):
    return jax.nn.softmax(x, axis=axis)
def _gelu(x):
    return jax.nn.gelu(x, approximate=True)
def _silu(x):
    return jax.nn.silu(x)
def _sigmoid(x):
    return jax.nn.sigmoid(x)
def _layernorm(x, axis=-1, eps=1e-5):
    m = jnp.mean(x, axis=axis, keepdims=True)
    v = jnp.var(x, axis=axis, keepdims=True)
    return (x - m) / jnp.sqrt(v + eps)
def _scatter_add(tgt, idx, src, axis=0):
    return tgt.at[idx].add(src)
def _segment_sum(src, seg, n):
    return jax.ops.segment_sum(src, seg, n)
class _Rng:
    def __init__(self, key):
        self._k = key
    def _next(self):
        self._k, sub = jax.random.split(self._k)
        return sub
    def normal(self, shape):
        return jax.random.normal(self._next(), shape, dtype=jnp.bfloat16)
    def randint(self, lo, hi, shape):
        return jax.random.randint(self._next(), shape, lo, hi, dtype=jnp.int32)
    def uniform(self, shape, lo=0.0, hi=1.0):
        return jax.random.uniform(self._next(), shape, jnp.bfloat16, lo, hi)
    def permutation(self, n):
        return jax.random.permutation(self._next(), n)


kernel_name = 'recurrent_scan__sliding_local_dilated__moe_arch_mod__prompt'

def setup_inputs():
    _rng = _Rng(jax.random.key(int.from_bytes(__import__("os").urandom(4), "little")))
    _w = (lambda a: (lambda t: t.astype(jnp.bfloat16) if jnp.issubdtype(t.dtype, jnp.floating) else t)(jnp.asarray(a)))
    def _A_setup():
        B, S, D = 1, 2048, 640
        return {
            "x": _w((lambda *s: _rng.normal(s) * 0.05)(B, S, D)),
            "wqkv": _w((lambda *s: _rng.normal(s) * 0.05)(D, 3 * D)),
            "wo": _w((lambda *s: _rng.normal(s) * 0.05)(D, D)),
        }
    _A_in = _A_setup()

    def _B_setup():
        B, S, D, F, C = 1, 2048, 640, 1728, 2
        return {
            "x": _w((lambda *s: _rng.normal(s) * 0.05)(B, S, D)),
            "w_r": _w((lambda *s: _rng.normal(s) * 0.05)(D)),
            "w_gate": _w((lambda *s: _rng.normal(s) * 0.05)(D, F)),
            "w_up": _w((lambda *s: _rng.normal(s) * 0.05)(D, F)),
            "w_down": _w((lambda *s: _rng.normal(s) * 0.05)(F, D)),
        }
    _B_in = _B_setup()

    return {
        "A_x": _A_in["x"],
        "A_wqkv": _A_in["wqkv"],
        "A_wo": _A_in["wo"],
        "B_x": _B_in["x"],
        "B_w_r": _B_in["w_r"],
        "B_w_gate": _B_in["w_gate"],
        "B_w_up": _B_in["w_up"],
        "B_w_down": _B_in["w_down"],
    }

def reference(A_x, A_wqkv, A_wo, B_x, B_w_r, B_w_gate, B_w_up, B_w_down):
    def _A_ref(x, wqkv, wo):
        B, S, D = x.shape
        H = 32; Dh = D // H
        W, dil = 8, 2
        qkv = (lambda x, *d: x.transpose(*d))((x @ wqkv).reshape(B, S, 3, H, Dh), 2, 0, 3, 1, 4)
        q, k, v = qkv[0], qkv[1], qkv[2]
        scale = Dh ** -0.5
        pos = jnp.arange(S)
        off = jnp.arange(W) * dil
        idx = pos[:, None] - off[None, :]
        mask = idx >= 0
        idx_c = jnp.where(mask, idx, 0).reshape(-1)
        kg = k[:, :, idx_c, :].reshape(B, H, S, W, Dh)
        vg = v[:, :, idx_c, :].reshape(B, H, S, W, Dh)
        logits = jnp.einsum("bhsd,bhswd->bhsw", q, kg) * scale
        logits = jnp.where(mask[None, None, :, :], logits, -1e9)
        attn = _softmax(logits, axis=-1)
        o = jnp.einsum("bhsw,bhswd->bhsd", attn, vg)
        return (lambda x, *d: x.transpose(*d))(o, 0, 2, 1, 3).reshape(B, S, D) @ wo

    def _B_ref(x, w_r, w_gate, w_up, w_down):
        B, S, D = x.shape
        C = 2
        r = x @ w_r
        idx = jnp.argsort(-r, axis=-1)[:, :C]
        idx_e = jnp.repeat(idx.reshape(B, C, 1), D, axis=2)
        x_sel = jnp.take_along_axis(x, idx_e, axis=1)
        g = _silu(x_sel @ w_gate)
        u = x_sel @ w_up
        y = (g * u) @ w_down
        r_sel = _sigmoid(jnp.take_along_axis(r, idx, axis=1))
        y = y * r_sel.reshape(B, C, 1)
        b_off = (jnp.arange(B) * S).reshape(B, 1)
        flat_idx = (idx + b_off).reshape(B * C)
        zero = (x * 0.0).reshape(B * S, D)
        upd = _scatter_add(zero, flat_idx, y.reshape(B * C, D), axis=0)
        return x + upd.reshape(B, S, D)

    x = A_x
    xn = _layernorm(x, axis=-1)
    s = _A_ref(xn, A_wqkv, A_wo)
    g = _silu(_B_ref(xn, B_w_r, B_w_gate, B_w_up, B_w_down))
    return x + s * g
```

```python
import functools

import jax
import jax.numpy as jnp
from jax import lax
from jax.experimental import pallas as pl
from jax.experimental.pallas import tpu as pltpu

F32 = jnp.float32
BF16 = jnp.bfloat16
I32 = jnp.int32

H = 32
W = 8
DIL = 2
HALO = 16
LOG2E = 1.4426950408889634


def _interleave(*gens):
    gens = [[g, float(n), 0] for g, n in gens]
    while gens:
        s = min(gens, key=lambda e: (e[2] + 0.5) / e[1])
        try:
            next(s[0])
            s[2] += 1
        except StopIteration:
            gens.remove(s)


def _run(g):
    for _ in g:
        pass


def _pipeline(items, make_gen):
    active = []
    items = list(items)
    while items or active:
        if items:
            active.insert(0, make_gen(items.pop(0)))
        for g in list(active):
            try:
                next(g)
            except StopIteration:
                active.remove(g)
        yield


def _kernel(x_hbm, wqkv_hbm, wo_hbm, wr_hbm, wg_hbm, wu_hbm, wd_hbm, out_hbm,
            x_v, wraw, wp, wo_raw, wo_f32, wop, wr_v, wrb, wg_v, wu_v, wd_v,
            xn_v, q0, k0, v0, q1, k1, v1, o_v, r_v, out_v,
            sem_x, sem_w, sem_m, sem_o, *, S, D, T, NCH, agap, lgap, scopes):
    NB = S // T
    NT = D // 128
    DH = D // H
    scale = DH ** -0.5
    bufs = ((q0, k0, v0), (q1, k1, v1))

    def row0(b, n=T):
        return b * n if isinstance(b, int) else pl.multiple_of(b * n, n)

    def x_copy(b):
        return pltpu.make_async_copy(x_hbm.at[pl.ds(b * T, T)], x_v.at[pl.ds(b * T, T)], sem_x.at[b])

    def w_copy(p):
        return pltpu.make_async_copy(wqkv_hbm.at[:, pl.ds(p * D, D)], wraw.at[p], sem_w.at[p])

    wr_copy = pltpu.make_async_copy(wr_hbm, wr_v, sem_m.at[0])
    wo_copy = pltpu.make_async_copy(wo_hbm, wo_raw, sem_m.at[1])
    wg_copy = pltpu.make_async_copy(wg_hbm, wg_v, sem_m.at[2])
    wu_copy = pltpu.make_async_copy(wu_hbm, wu_v, sem_m.at[3])
    wd_copy = pltpu.make_async_copy(wd_hbm, wd_v, sem_m.at[4])

    def o_copy(b):
        r0 = row0(b)
        return pltpu.make_async_copy(out_v.at[pl.ds(r0, T)], out_hbm.at[pl.ds(r0, T)], sem_o.at[b])

    x_copy(0).start()
    wr_copy.start()
    w_copy(0).start()

    lane = lax.broadcasted_iota(I32, (8, 128), 1)
    sub = lax.broadcasted_iota(I32, (8, 128), 0)

    def permute_w(p):
        quad = lane >> 2
        for e in range(NT):
            hh = ((quad - e) * 13) & 31
            src_tile = (5 * hh + e) >> 5
            gidx = (20 * (lane & 31) + 4 * e + (lane >> 5)) & 127
            for r in range(0, D, 16):
                u = None
                for t in range(NT):
                    a = pltpu.bitcast(wraw[p, pl.ds(r, 16), pl.ds(t * 128, 128)], I32)
                    u = a if u is None else jnp.where(src_tile == t, a, u)
                wp[pl.ds(r // 2, 8), pl.ds(p * D + e * 128, 128)] = jnp.take_along_axis(u, gidx, axis=1)

    def permute_wo():
        for t in range(NT):
            wo_f32[t] = wo_raw[:, pl.ds(t * 128, 128)].astype(F32)
            yield
        for t in range(NT):
            for d in range(DH):
                wop[pl.ds(d * H // 2, H // 2), pl.ds(t * 128, 128)] = pltpu.bitcast(
                    wo_f32[t, pl.ds(d, H, stride=DH), :].astype(BF16), I32)
            yield

    def rb(a):
        return a.astype(BF16).astype(F32)

    def layernorm(b):
        r0 = row0(b)
        h0 = row0(b, T // 2)
        racc = [jnp.zeros((8, 128), F32)]

        def rows(g):
            xb = x_v[pl.ds(r0 + g * 16, 16), :].astype(F32)
            mean = jnp.sum(xb, axis=-1, keepdims=True) * (1.0 / D)
            for _ in range(lgap):
                yield
            mb = rb(mean)
            c = x_v[pl.ds(r0 + g * 16, 16), :].astype(F32) - mb
            dm = mean - mb
            var = jnp.sum(c * c, axis=-1, keepdims=True)
            for _ in range(lgap):
                yield
            var = jnp.maximum(var * (1.0 / D) - dm * dm, 0.0)
            den = rb(jnp.sqrt(rb(rb(var) + rb(jnp.full_like(var, 1e-5)))))
            xn = c * (1.0 / den)
            xn_v[pl.ds(h0 + g * 8, 8), :] = pltpu.bitcast(xn.astype(BF16), I32)
            wrow = wrb[...]
            rr = [jnp.sum(xn[hf * 8:(hf + 1) * 8] * wrow, axis=-1, keepdims=True) for hf in range(2)]
            for _ in range(lgap):
                yield
            for hf in range(2):
                racc[0] = jnp.where(lane == (2 * g + hf), rr[hf], racc[0])

        yield from _pipeline(range(T // 16), rows)
        r_v[b] = racc[0]

    def qkv(b, slot, c_lo=0, c_hi=3 * NT):
        h0 = row0(b, T // 2)
        qd, kd, vd = bufs[slot]
        dst = [(qd, e, 0) for e in range(NT)] + [(kd, e, HALO) for e in range(NT)] + [(vd, e, HALO) for e in range(NT)]
        for c0 in range(c_lo, c_hi, NCH):
            n = min(NCH, c_hi - c0)
            xb = pltpu.bitcast(xn_v[pl.ds(h0, T // 2), :], BF16)
            wb = pltpu.bitcast(wp[:, pl.ds(c0 * 128, n * 128)], BF16)
            res = jnp.dot(xb, wb, preferred_element_type=F32)
            for j in range(n):
                ref, e, off = dst[c0 + j]
                ref[e, pl.ds(off, T), :] = res[:, j * 128:(j + 1) * 128]
            yield

    n_qkv = -(-3 * NT // NCH)

    def halo(src, dst):
        for e in range(NT):
            bufs[dst][1][e, pl.ds(0, HALO), :] = bufs[src][1][e, pl.ds(T, HALO), :]
            bufs[dst][2][e, pl.ds(0, HALO), :] = bufs[src][2][e, pl.ds(T, HALO), :]

    def attention(b, slot):
        r0 = row0(b)
        h0 = row0(b, T // 2)
        q_v, k_v, v_v = bufs[slot]
        held = {}

        def rows(r):
            q = [q_v[e, pl.ds(r, 8), :] for e in range(NT)]
            ls = []
            for w in range(W):
                a = None
                for e in range(NT):
                    t = q[e] * k_v[e, pl.ds(HALO + r - DIL * w, 8), :]
                    a = t if a is None else a + t
                ls.append(a)
            rs = [pltpu.roll(a, 64, 1) for a in ls]
            for _ in range(agap):
                yield
            ls = [a + c for a, c in zip(ls, rs)]
            rs = [pltpu.roll(a, 32, 1) for a in ls]
            for _ in range(agap):
                yield
            ls = [a + c for a, c in zip(ls, rs)]
            for w in range(W):
                if r - DIL * w < 0 and not (isinstance(b, int) and b > 0):
                    ls[w] = jnp.where(sub + (r0 + r - DIL * w) >= 0, ls[w], -1e9 / scale)
            m = ls[0]
            for w in range(1, W):
                m = jnp.maximum(m, ls[w])
            ps = [jnp.exp2((l - m) * (scale * LOG2E)) for l in ls]
            s = ps[0]
            for w in range(1, W):
                s = s + ps[w]
            inv = 1.0 / s
            o = []
            for e in range(NT):
                a = None
                for w in range(W):
                    t = ps[w] * v_v[e, pl.ds(HALO + r - DIL * w, 8), :]
                    a = t if a is None else a + t
                o.append(a * inv)
            if r % 16 == 0:
                held[r] = o
                return
            prev = held.pop(r - 8)
            for e in range(NT):
                o_v[pl.ds(h0 + (r - 8) // 2, 8), pl.ds(e * 128, 128)] = pltpu.bitcast(
                    jnp.concatenate([prev[e], o[e]], axis=0).astype(BF16), I32)

        yield from _pipeline(range(0, T, 8), rows)

    def routed_ffn():
        big = S
        rs, toks = [], []
        for b in range(NB):
            valid = lane < (T // 8)
            rs.append(jnp.where(valid, rb(r_v[b]), -jnp.inf))
            toks.append(jnp.where(valid, b * T + lane * 8 + sub, big))

        def top(rs):
            m = rs[0]
            for a in rs[1:]:
                m = jnp.maximum(m, a)
            mx = jnp.max(jnp.max(m, axis=1, keepdims=True), axis=0, keepdims=True)
            c = None
            for a, t in zip(rs, toks):
                cc = jnp.where(a == mx, t, big)
                c = cc if c is None else jnp.minimum(c, cc)
            cf = c.astype(F32)
            ix = jnp.min(jnp.min(cf, axis=1, keepdims=True), axis=0, keepdims=True).astype(I32)
            return mx, ix

        m0, i0 = top(rs)
        rs2 = [jnp.where(t == i0, -jnp.inf, a) for a, t in zip(rs, toks)]
        m1, i1 = top(rs2)
        idx = [jnp.clip(i0[0, 0], 0, S - 1), jnp.clip(i1[0, 0], 0, S - 1)]
        row16 = lax.broadcasted_iota(I32, (16, D), 0)
        bases = [pl.multiple_of((i >> 4) << 3, 8) for i in idx]
        sel = []
        for j in range(2):
            tile = pltpu.bitcast(xn_v[pl.ds(bases[j], 8), :], BF16).astype(F32)
            sel.append(jnp.sum(jnp.where(row16 == (idx[j] & 15), tile, 0.0), axis=0, keepdims=True))
        xs = jnp.where(row16 == 0, sel[0], jnp.where(row16 == 1, sel[1], 0.0)).astype(BF16)
        nt = (((1,), (1,)), ((), ()))
        yield
        gt = rb(lax.dot_general(xs, wg_v[...], nt, preferred_element_type=F32))
        yield
        up = rb(lax.dot_general(xs, wu_v[...], nt, preferred_element_type=F32))
        hid = (rb(gt * jax.nn.sigmoid(gt)) * up).astype(BF16)
        yield
        y = rb(jnp.dot(hid, wd_v[...], preferred_element_type=F32))
        for j, m in enumerate((m0, m1)):
            yj = rb(y[j:j + 1, :] * rb(jax.nn.sigmoid(m)))
            tile = pltpu.bitcast(xn_v[pl.ds(bases[j], 8), :], BF16).astype(F32)
            tile = jnp.where(row16 == (idx[j] & 15), tile + yj, tile)
            xn_v[pl.ds(bases[j], 8), :] = pltpu.bitcast(tile.astype(BF16), I32)
        yield

    def out_proj(b):
        r0 = row0(b)
        h0 = row0(b, T // 2)
        s = jnp.dot(pltpu.bitcast(o_v[pl.ds(h0, T // 2), :], BF16), pltpu.bitcast(wop[...], BF16),
                    preferred_element_type=F32)
        hz = pltpu.bitcast(xn_v[pl.ds(h0, T // 2), :], BF16).astype(F32) * 0.5
        gate = hz * jnp.tanh(hz) + hz
        out_v[pl.ds(r0, T), :] = (x_v[pl.ds(r0, T), :].astype(F32) + s * gate).astype(BF16)
        o_copy(b).start()
        yield

    G = T // 16
    import contextlib
    ns = jax.named_scope if scopes else (lambda n: contextlib.nullcontext())
    with ns("p0_wait"):
        wr_copy.wait()
        wrb[...] = jnp.broadcast_to(wr_v[...].astype(F32).reshape(1, D), (8, D))
        x_copy(0).wait()
        w_copy(1).start()
    with ns("p1_ln0"):
        _run(layernorm(0))
    with ns("p2_w0"):
        w_copy(0).wait()
        w_copy(2).start()
    with ns("p3_perm0"):
        permute_w(0)
    with ns("p4_w1"):
        w_copy(1).wait()
        x_copy(1).start()
    with ns("p5_dot0"):
        _run(qkv(0, 0, 0, NT))
        permute_w(1)
    with ns("p6_w2"):
        w_copy(2).wait()
        for b in range(2, NB):
            x_copy(b).start()
        x_copy(1).wait()
    with ns("s0"):
        _run(qkv(0, 0, NT, 2 * NT))
        permute_w(2)
        _run(qkv(0, 0, 2 * NT, 3 * NT))
        _run(layernorm(1))
        for e in range(NT):
            k0[e, pl.ds(0, HALO), :] = jnp.zeros((HALO, 128), F32)
            v0[e, pl.ds(0, HALO), :] = jnp.broadcast_to(v0[e, pl.ds(HALO, 1), :], (HALO, 128))
    wo_copy.start()
    wg_copy.start()
    wu_copy.start()
    wd_copy.start()
    for i in range(1, NB):
        slot = i & 1
        with ns(f"s{i}"):
            if i + 1 < NB:
                x_copy(i + 1).wait()
            else:
                wo_copy.wait()
            halo(1 - slot, slot)
            _run(qkv(i, slot))
            _run(attention(i - 1, 1 - slot))
            if i + 1 < NB:
                _run(layernorm(i + 1))
            else:
                _run(permute_wo())
    with ns("t0_wait"):
        wg_copy.wait()
        wu_copy.wait()
        wd_copy.wait()
    with ns("t1_rest"):
        _run(routed_ffn())
        _run(attention(NB - 1, (NB - 1) & 1))
        for i in range(NB):
            _run(out_proj(i))
    with ns("t2_owait"):
        for b in range(NB):
            o_copy(b).wait()


def make(T=256, NCH=15, agap=1, lgap=1, flags={"XLA_TPU_EVENLY_DISTRIBUTE_CRITICAL_NODES":True}, scopes=False, name="fused"):
    @jax.jit
    def fn(A_x, A_wqkv, A_wo, B_x, B_w_r, B_w_gate, B_w_up, B_w_down):
        del B_x
        Bn, S, D = A_x.shape
        Fd = B_w_gate.shape[1]
        NB = S // T
        NT = D // 128
        any_spec = pl.BlockSpec(memory_space=pltpu.HBM)
        qkv_bufs = [
            pltpu.VMEM((NT, T, 128), F32),
            pltpu.VMEM((NT, T + HALO, 128), F32),
            pltpu.VMEM((NT, T + HALO, 128), F32),
        ]
        out = pl.pallas_call(
            functools.partial(_kernel, S=S, D=D, T=T, NCH=NCH, agap=agap, lgap=lgap, scopes=scopes),
            in_specs=[any_spec] * 7,
            out_specs=any_spec,
            out_shape=jax.ShapeDtypeStruct((S, D), A_x.dtype),
            scratch_shapes=[
                pltpu.VMEM((S, D), BF16),
                pltpu.VMEM((3, D, D), BF16),
                pltpu.VMEM((D // 2, 3 * D), I32),
                pltpu.VMEM((D, D), BF16),
                pltpu.VMEM((NT, D, 128), F32),
                pltpu.VMEM((D // 2, D), I32),
                pltpu.VMEM((D,), BF16),
                pltpu.VMEM((8, D), F32),
                pltpu.VMEM((Fd, D), BF16),
                pltpu.VMEM((Fd, D), BF16),
                pltpu.VMEM((Fd, D), BF16),
                pltpu.VMEM((S // 2, D), I32),
                *qkv_bufs, *qkv_bufs,
                pltpu.VMEM((S // 2, D), I32),
                pltpu.VMEM((NB, 8, 128), F32),
                pltpu.VMEM((S, D), BF16),
                pltpu.SemaphoreType.DMA((NB,)),
                pltpu.SemaphoreType.DMA((3,)),
                pltpu.SemaphoreType.DMA((5,)),
                pltpu.SemaphoreType.DMA((NB,)),
            ],
            compiler_params=pltpu.CompilerParams(vmem_limit_bytes=100 * 2**20, flags=flags),
            name=name,
        )(A_x.reshape(S, D), A_wqkv, A_wo, B_w_r, B_w_gate.T, B_w_up.T, B_w_down)
        return out.reshape(Bn, S, D)
    return fn


_impl = make()


@jax.jit
def pallas_recurrent_scan__sliding_local_dilated__moe_arch_mod__prompt_kernel(
        A_x, A_wqkv, A_wo, B_x, B_w_r, B_w_gate, B_w_up, B_w_down):
    return _impl(A_x, A_wqkv, A_wo, B_x, B_w_r, B_w_gate, B_w_up, B_w_down)
```

```python
import contextlib
import functools

import jax
import jax.numpy as jnp
from jax import lax
from jax.experimental import pallas as pl
from jax.experimental.pallas import tpu as pltpu

F32 = jnp.float32
BF16 = jnp.bfloat16
I32 = jnp.int32

H = 32
W = 8
DIL = 2
HALO = 16
LOG2E = 1.4426950408889634
NT_DIMS = (((1,), (1,)), ((), ()))


def _run(g):
    for _ in g:
        pass


def _zip(*gens):
    gens = list(gens)
    while gens:
        for g in list(gens):
            try:
                next(g)
            except StopIteration:
                gens.remove(g)


def _take(g, n):
    for _ in range(n):
        next(g)
        yield


def _alt(a, b, split):
    for _ in a:
        if split > 1:
            yield
        next(b)
        yield


def _chain(*gens):
    for g in gens:
        yield from g


def _pipeline(items, make_gen):
    active = []
    items = list(items)
    while items or active:
        if items:
            active.insert(0, make_gen(items.pop(0)))
        for g in list(active):
            try:
                next(g)
            except StopIteration:
                active.remove(g)
        yield


def _rb(a):
    return a.astype(BF16).astype(F32)


def _silu(z):
    h = 0.5 * z
    return h * jnp.tanh(h) + h


def _kernel(x_hbm, wqkv_hbm, wo_hbm, wr_hbm, wg_hbm, wu_hbm, wd_hbm, out_hbm,
            x_v, wraw, wp, wo_raw, wo_f32, wop, wr_v, wrb, wg_v, wu_v, wd_v,
            xn_v, q0, k0, v0, q1, k1, v1, o_v, s_v, out_v,
            sem_i, sem_o, sem_f, *, S, D, T, scopes, opt):
    NB = S // T
    NT = D // 128
    DH = D // H
    FF = wg_v.shape[0]
    NF = -(-FF // 128)
    scale = DH ** -0.5
    bufs = ((q0, k0, v0), (q1, k1, v1))

    def x_copy(b):
        return pltpu.make_async_copy(x_hbm.at[pl.ds(b * T, T)], x_v.at[pl.ds(b * T, T)], sem_i.at[b])

    def w_copy(c):
        return pltpu.make_async_copy(wqkv_hbm.at[pl.ds(c * 128, 128)], wraw.at[c], sem_i.at[NB + c])

    wr_copy = pltpu.make_async_copy(wr_hbm, wr_v, sem_i.at[NB + NT])
    wo_copy = pltpu.make_async_copy(wo_hbm, wo_raw, sem_i.at[NB + NT + 1])
    wg_copy = pltpu.make_async_copy(wg_hbm, wg_v, sem_i.at[NB + NT + 2])
    wu_copy = pltpu.make_async_copy(wu_hbm, wu_v, sem_i.at[NB + NT + 3])
    wd_copy = pltpu.make_async_copy(wd_hbm, wd_v, sem_i.at[NB + NT + 4])

    out_parts = [(b * T, T) for b in range(NB - 1)]
    r = (NB - 1) * T
    for n in opt.get("last", (T,)):
        out_parts.append((r, n))
        r += n

    def o_copy(j):
        r0, n = out_parts[j]
        return pltpu.make_async_copy(out_v.at[pl.ds(r0, n)], out_hbm.at[pl.ds(r0, n)], sem_o.at[j])

    wr_copy.start()
    x_copy(0).start()
    for c in range(NT):
        w_copy(c).start()
    for b in range(1, NB):
        x_copy(b).start()
    wo_copy.start()
    wg_copy.start()
    wu_copy.start()
    wd_copy.start()

    lane = lax.broadcasted_iota(I32, (8, 128), 1)
    sub = lax.broadcasted_iota(I32, (8, 128), 0)

    def permute_w(c):
        quad = lane >> 2
        src_tile = [(5 * (((quad - e) * 13) & 31) + e) >> 5 for e in range(NT)]
        gidx = [(20 * (lane & 31) + 4 * e + (lane >> 5)) & 127 for e in range(NT)]
        nb = opt.get("pb", 0)
        for p in range(3):
            for r0 in range(0, 128, 16 * max(nb, 1)):
                a = {r: [pltpu.bitcast(wraw[c, pl.ds(r, 16), pl.ds(p * D + t * 128, 128)], I32) for t in range(NT)]
                     for r in range(r0, r0 + 16 * max(nb, 1), 16)}
                for e in range(NT):
                    for r in a:
                        u = a[r][0]
                        for t in range(1, NT):
                            u = jnp.where(src_tile[e] == t, a[r][t], u)
                        if nb:
                            u = jnp.take_along_axis(u, gidx[e], axis=1)
                        wp[pl.ds(c * 64 + r // 2, 8), pl.ds(p * D + e * 128, 128)] = u
        if not nb:
            for e in range(NT):
                for p in range(3):
                    for r in range(0, 64, 8):
                        at = (pl.ds(c * 64 + r, 8), pl.ds(p * D + e * 128, 128))
                        wp[at] = jnp.take_along_axis(wp[at], gidx[e], axis=1)

    def permute_wo(t):
        wo_f32[t] = wo_raw[:, pl.ds(t * 128, 128)].astype(F32)
        for d in range(DH):
            wop[pl.ds(d * H // 2, H // 2), pl.ds(t * 128, 128)] = pltpu.bitcast(
                wo_f32[t, pl.ds(d, H, stride=DH), :].astype(BF16), I32)

    score = [jnp.zeros((8, 128), F32) for _ in range(S // 1024)]

    def layernorm(g_lo, g_hi):
        def rows(g):
            xb = x_v[pl.ds(g * 16, 16), :].astype(F32)
            mean = jnp.sum(xb, axis=-1, keepdims=True) * (1.0 / D)
            yield
            mb = _rb(mean)
            c = x_v[pl.ds(g * 16, 16), :].astype(F32) - mb
            dm = mean - mb
            var = jnp.sum(c * c, axis=-1, keepdims=True)
            yield
            var = jnp.maximum(var * (1.0 / D) - dm * dm, 0.0)
            ve = _rb(_rb(var) + _rb(jnp.full_like(var, 1e-5)))
            den = _rb(ve * lax.rsqrt(ve))
            xn = c * pltpu.reciprocal(den, approx=True)
            xn_v[pl.ds(g * 8, 8), :] = pltpu.bitcast(xn.astype(BF16), I32)
            wrow = wrb[...]
            rr = [jnp.sum(xn[hf * 8:(hf + 1) * 8] * wrow, axis=-1, keepdims=True) for hf in range(2)]
            yield
            for hf in range(2):
                j = 2 * g + hf
                score[j // 128] = jnp.where(lane == (j % 128), rr[hf], score[j // 128])

        _run(_pipeline(range(g_lo, g_hi), rows))

    def qkv_dst(slot):
        qd, kd, vd = bufs[slot]
        return [(qd, e, 0) for e in range(NT)] + [(kd, e, HALO) for e in range(NT)] + [(vd, e, HALO) for e in range(NT)]

    def qkv(b):
        dst = qkv_dst(b & 1)
        xb = pltpu.bitcast(xn_v[pl.ds(b * T // 2, T // 2), :], BF16)
        res = jnp.dot(xb, pltpu.bitcast(wp[...], BF16), preferred_element_type=F32)
        for j, (ref, e, off) in enumerate(dst):
            ref[e, pl.ds(off, T), :] = res[:, j * 128:(j + 1) * 128]

    def qkv_pieces(b, split=1):
        m = T // split
        for j, (ref, e, off) in enumerate(qkv_dst(b & 1)):
            for r in range(0, T, m):
                xb = pltpu.bitcast(xn_v[pl.ds((b * T + r) // 2, m // 2), :], BF16)
                ref[e, pl.ds(off + r, m), :] = jnp.dot(xb, pltpu.bitcast(wp[:, pl.ds(j * 128, 128)], BF16),
                                                       preferred_element_type=F32)
                yield

    def qkv_first(c):
        xb = pltpu.bitcast(xn_v[pl.ds(0, T // 2), pl.ds(c * 128, 128)], BF16)
        res = jnp.dot(xb, pltpu.bitcast(wp[pl.ds(c * 64, 64), :], BF16), preferred_element_type=F32)
        for j, (ref, e, off) in enumerate(qkv_dst(0)):
            part = res[:, j * 128:(j + 1) * 128]
            if c > 0:
                part = part + ref[e, pl.ds(off, T), :]
            ref[e, pl.ds(off, T), :] = part

    def halo(src, dst):
        for e in range(NT):
            bufs[dst][1][e, pl.ds(0, HALO), :] = bufs[src][1][e, pl.ds(T, HALO), :]
            bufs[dst][2][e, pl.ds(0, HALO), :] = bufs[src][2][e, pl.ds(T, HALO), :]

    def attention(b):
        q_v, k_v, v_v = bufs[b & 1]
        held = {}

        def rows(r):
            q = [q_v[e, pl.ds(r, 8), :] for e in range(NT)]
            ls = []
            for w in range(W):
                a = None
                for e in range(NT):
                    t = q[e] * k_v[e, pl.ds(HALO + r - DIL * w, 8), :]
                    a = t if a is None else a + t
                ls.append(a)
            rs = [pltpu.roll(a, 64, 1) for a in ls]
            yield
            ls = [a + c for a, c in zip(ls, rs)]
            rs = [pltpu.roll(a, 32, 1) for a in ls]
            yield
            ls = [a + c for a, c in zip(ls, rs)]
            for w in range(W):
                if b * T + r - DIL * w < 0:
                    ls[w] = jnp.where(sub + (b * T + r - DIL * w) >= 0, ls[w], -1e9 / scale)
            m = ls[0]
            for w in range(1, W):
                m = jnp.maximum(m, ls[w])
            ps = [jnp.exp2((l - m) * (scale * LOG2E)) for l in ls]
            s = ps[0]
            for w in range(1, W):
                s = s + ps[w]
            inv = pltpu.reciprocal(s, approx=True)
            o = []
            for e in range(NT):
                a = None
                for w in range(W):
                    t = ps[w] * v_v[e, pl.ds(HALO + r - DIL * w, 8), :]
                    a = t if a is None else a + t
                o.append(a * inv)
            if r % 16 == 0:
                held[r] = o
                return
            prev = held.pop(r - 8)
            for e in range(NT):
                o_v[pl.ds((b * T + r - 8) // 2, 8), pl.ds(e * 128, 128)] = pltpu.bitcast(
                    jnp.concatenate([prev[e], o[e]], axis=0).astype(BF16), I32)

        _run(_pipeline(range(0, T, 8), rows))

    row16 = lax.broadcasted_iota(I32, (16, D), 0)

    def route():
        rs = [_rb(a) for a in score]
        toks = [((j * 128 + lane) * 8 + sub).astype(F32) for j in range(len(rs))]

        def top(rs):
            m = functools.reduce(jnp.maximum, rs)
            mx = jnp.max(jnp.max(m, axis=1, keepdims=True), axis=0, keepdims=True)
            c = functools.reduce(jnp.minimum, [jnp.where(a == mx, t, float(S)) for a, t in zip(rs, toks)])
            return mx, jnp.min(jnp.min(c, axis=1, keepdims=True), axis=0, keepdims=True)

        m0, i0 = top(rs)
        m1, i1 = top([jnp.where(t == i0, -jnp.inf, a) for a, t in zip(rs, toks)])
        idx = [jnp.clip(i.astype(I32)[0, 0], 0, S - 1) for i in (i0, i1)]
        sel = []
        for i in idx:
            tile = pltpu.bitcast(xn_v[pl.ds(pl.multiple_of((i >> 4) << 3, 8), 8), :], BF16).astype(F32)
            sel.append(jnp.sum(jnp.where(row16 == (i & 15), tile, 0.0), axis=0, keepdims=True))
        xs = jnp.where(row16 == 0, sel[0], jnp.where(row16 == 1, sel[1], 0.0)).astype(BF16)
        return xs, idx, (m0, m1)

    def ffn_in(xs, w_ref, res):
        for n0 in range(0, FF, 128):
            res.append(_rb(lax.dot_general(xs, w_ref[pl.ds(n0, min(128, FF - n0)), :], NT_DIMS,
                                           preferred_element_type=F32)))
            yield

    def ffn_out(hid, res):
        acc = None
        for j, n0 in enumerate(range(0, FF, 128)):
            t = jnp.dot(hid[j], wd_v[pl.ds(n0, min(128, FF - n0)), :], preferred_element_type=F32)
            acc = t if acc is None else acc + t
            if j == NF - 1:
                res.append(_rb(acc))
            yield

    def ffn_apply(y, idx, ms):
        for j, m in enumerate(ms):
            yj = _rb(y[j:j + 1, :] * _rb(1.0 / (1.0 + jnp.exp(-m))))
            at = pl.ds(pl.multiple_of((idx[j] >> 4) << 3, 8), 8)
            tile = pltpu.bitcast(xn_v[at, :], BF16).astype(F32)
            tile = jnp.where(row16 == (idx[j] & 15), tile + yj, tile)
            xn_v[at, :] = pltpu.bitcast(tile.astype(BF16), I32)

    def gate_tile(j, e, s):
        r0, n = out_parts[j]
        cols = pl.ds(e * 128, 128)
        for r in range(0, n, 32):
            z = pltpu.bitcast(xn_v[pl.ds((r0 + r) // 2, 16), cols], BF16).astype(F32)
            out_v[pl.ds(r0 + r, 32), cols] = (
                x_v[pl.ds(r0 + r, 32), cols].astype(F32) + s(r) * _silu(z)).astype(BF16)
            yield

    def out_tile(j, e):
        r0, n = out_parts[j]
        return jnp.dot(pltpu.bitcast(o_v[pl.ds(r0 // 2, n // 2), :], BF16),
                       pltpu.bitcast(wop[:, pl.ds(e * 128, 128)], BF16), preferred_element_type=F32)

    def out_proj_pieces(j):
        for e in range(NT):
            s_v[j, :, pl.ds(e * 128, 128)] = out_tile(j, e)
            yield

    def fence():
        pl.semaphore_signal(sem_f, 1)
        pl.semaphore_wait(sem_f, 1)

    def ns(n):
        return jax.named_scope(n) if scopes else contextlib.nullcontext()

    G = T // 16
    with ns("p0_wait"):
        wr_copy.wait()
        wrb[...] = jnp.broadcast_to(wr_v[...].astype(F32).reshape(1, D), (8, D))
    with ns("p1_ln0"):
        x_copy(0).wait()
        layernorm(0, G)
    with ns("p2_perm0"):
        w_copy(0).wait()
        permute_w(0)
    for c in range(NT - 1):
        with ns(f"p3_dot{c}"):
            w_copy(c + 1).wait()
            qkv_first(c)
            permute_w(c + 1)
    with ns("p4_dot4"):
        x_copy(1).wait()
        qkv_first(NT - 1)
        layernorm(G, 2 * G)
        for e in range(NT):
            k0[e, pl.ds(0, HALO), :] = jnp.zeros((HALO, 128), F32)
            v0[e, pl.ds(0, HALO), :] = jnp.broadcast_to(v0[e, pl.ds(HALO, 1), :], (HALO, 128))

    n_ln = NB - 3
    per = -(-(NB - 2) * G // n_ln)
    g_done, x_done = 2 * G, 2
    gt, up, y = [], [], []
    skip = opt.get("skip", ())
    for i in range(1, NB):
        with ns(f"s{i}"):
            g_next = min(g_done + (opt['ln'][i - 1] if 'ln' in opt and i <= n_ln else per), NB * G)
            fenced = False
            while x_done * G < (g_next if i == 1 else NB * G):
                x_copy(x_done).wait()
                x_done += 1
                fenced = True
            if i == 2:
                wo_copy.wait()
            if i == NB - 2:
                wg_copy.wait()
                wu_copy.wait()
            elif i == NB - 1:
                wd_copy.wait()
            elif not fenced and i not in skip:
                fence()
            halo(1 - (i & 1), i & 1)
            if i == NB - 2:
                _zip(qkv_pieces(i, opt.get("msplit", 1)), _alt(ffn_in(xs, wg_v, gt), ffn_in(xs, wu_v, up), opt.get("msplit", 1)))
            elif i == NB - 1:
                hid = [(_rb(_silu(g)) * u).astype(BF16) for g, u in zip(gt, up)]
                _zip(qkv_pieces(i), ffn_out(hid, y))
            else:
                qkv(i)
            if i == n_ln:
                layernorm(g_done, g_next)
                xs, idx, ms = route()
            attention(i - 1)
            if i < n_ln:
                layernorm(g_done, g_next)
            g_done = g_next
            for t in range(NT):
                if opt.get("wo_at", (3, 4, 5, 6, 7))[t] == i:
                    permute_wo(t)
    with ns("t0"):
        fence()
        ffn_apply(y[0], idx, ms)
        attention(NB - 1)
        for j in range(len(out_parts)):
            if j in opt.get("tf", ()):
                fence()
            if opt.get("whole"):
                r0, n = out_parts[j]
                full = jnp.dot(pltpu.bitcast(o_v[pl.ds(r0 // 2, n // 2), :], BF16), pltpu.bitcast(wop[...], BF16),
                               preferred_element_type=F32)
            for e in range(NT):
                t = full[:, e * 128:(e + 1) * 128] if opt.get("whole") else out_tile(j, e)
                _run(gate_tile(j, e, lambda r: t[r:r + 32]))
            o_copy(j).start()
    with ns("t2_owait"):
        for j in range(len(out_parts)):
            o_copy(j).wait()


def make(T=256, flags={"XLA_TPU_EVENLY_DISTRIBUTE_CRITICAL_NODES": True}, scopes=False, name="fused", **opt):
    @jax.jit
    def fn(A_x, A_wqkv, A_wo, B_x, B_w_r, B_w_gate, B_w_up, B_w_down):
        del B_x
        Bn, S, D = A_x.shape
        Fd = B_w_gate.shape[1]
        NB = S // T
        NT = D // 128
        hbm = pl.BlockSpec(memory_space=pltpu.HBM)
        qkv_bufs = [
            pltpu.VMEM((NT, T, 128), F32),
            pltpu.VMEM((NT, T + HALO, 128), F32),
            pltpu.VMEM((NT, T + HALO, 128), F32),
        ]
        out = pl.pallas_call(
            functools.partial(_kernel, S=S, D=D, T=T, scopes=scopes, opt=opt),
            in_specs=[hbm] * 7,
            out_specs=hbm,
            out_shape=jax.ShapeDtypeStruct((S, D), A_x.dtype),
            scratch_shapes=[
                pltpu.VMEM((S, D), BF16),
                pltpu.VMEM((NT, 128, 3 * D), BF16),
                pltpu.VMEM((D // 2, 3 * D), I32),
                pltpu.VMEM((D, D), BF16),
                pltpu.VMEM((NT, D, 128), F32),
                pltpu.VMEM((D // 2, D), I32),
                pltpu.VMEM((D,), BF16),
                pltpu.VMEM((8, D), F32),
                pltpu.VMEM((Fd, D), BF16),
                pltpu.VMEM((Fd, D), BF16),
                pltpu.VMEM((Fd, D), BF16),
                pltpu.VMEM((S // 2, D), I32),
                *qkv_bufs, *qkv_bufs,
                pltpu.VMEM((S // 2, D), I32),
                pltpu.VMEM((3, T, D), F32),
                pltpu.VMEM((S, D), BF16),
                pltpu.SemaphoreType.DMA((NB + NT + 5,)),
                pltpu.SemaphoreType.DMA((NB + 4,)),
                pltpu.SemaphoreType.REGULAR,
            ],
            compiler_params=pltpu.CompilerParams(vmem_limit_bytes=100 * 2**20, flags=flags),
            name=name,
        )(A_x.reshape(S, D), A_wqkv, A_wo, B_w_r, B_w_gate.T, B_w_up.T, B_w_down)
        return out.reshape(Bn, S, D)
    return fn


_impl = make(pb=4, last=(192, 64), whole=1, msplit=2, tf=(3,), wo_at=(5, 6, 6, 7, 7), ln=(19, 19, 19, 19, 20))


@jax.jit
def pallas_recurrent_scan__sliding_local_dilated__moe_arch_mod__prompt_kernel(
        A_x, A_wqkv, A_wo, B_x, B_w_r, B_w_gate, B_w_up, B_w_down):
    return _impl(A_x, A_wqkv, A_wo, B_x, B_w_r, B_w_gate, B_w_up, B_w_down)
```

```python
import functools

import jax
import jax.numpy as jnp
from jax import lax
from jax.experimental import pallas as pl
from jax.experimental.pallas import tpu as pltpu

F32 = jnp.float32
BF16 = jnp.bfloat16
I32 = jnp.int32

H = 32
W = 8
DIL = 2
HALO = 16
LOG2E = 1.4426950408889634
NT_DIMS = (((1,), (1,)), ((), ()))

QKV_BLOCKS = (256, 448, 448, 448, 448)
LN_PARTS = (256, 128, 320, 832, 512)
OUT_PARTS = (256,) * 7 + (128, 64, 64)


def _run(g):
    for _ in g:
        pass


def _chain(*gens):
    for g in gens:
        yield from g


def _mix(*gens):
    gens = [[g, float(n), 0] for g, n in gens]
    while gens:
        s = min(gens, key=lambda e: e[2] / e[1])
        try:
            next(s[0])
            s[2] += 1
        except StopIteration:
            gens.remove(s)


def _pipeline(items, make_gen):
    active = []
    items = list(items)
    while items or active:
        if items:
            active.insert(0, make_gen(items.pop(0)))
        for g in list(active):
            try:
                next(g)
            except StopIteration:
                active.remove(g)
        yield


def _spans(sizes):
    out, r = [], 0
    for n in sizes:
        out.append((r, n))
        r += n
    return out


def _rb(a):
    return a.astype(BF16).astype(F32)


def _silu(z):
    h = 0.5 * z
    return h * jnp.tanh(h) + h


def _bf16(a):
    return pltpu.bitcast(a, BF16)


def _kernel(x_hbm, wqkv_hbm, wo_hbm, wr_hbm, wg_hbm, wu_hbm, wd_hbm, out_hbm,
            x_v, wraw, wp, wo_raw, wo_cols, wop, wr_v, wrb, wg_v, wu_v, wd_v,
            xn_v, q0, k0, v0, q1, k1, v1, o_v, out_v,
            sem_i, sem_o, sem_f):
    S, D = x_v.shape
    NT = D // 128
    DH = D // H
    FF = wg_v.shape[0]
    NF = -(-FF // 128)
    scale = DH ** -0.5
    bufs = ((q0, k0, v0), (q1, k1, v1))
    blocks = _spans(QKV_BLOCKS)
    x_parts = _spans(LN_PARTS)
    out_parts = _spans(OUT_PARTS)
    NX = len(x_parts)

    def x_copy(j):
        at = pl.ds(*x_parts[j])
        return pltpu.make_async_copy(x_hbm.at[at], x_v.at[at], sem_i.at[j])

    def w_copy(c):
        return pltpu.make_async_copy(wqkv_hbm.at[pl.ds(c * 128, 128)], wraw.at[c], sem_i.at[NX + c])

    wr_copy = pltpu.make_async_copy(wr_hbm, wr_v, sem_i.at[NX + NT])
    wo_copy = pltpu.make_async_copy(wo_hbm, wo_raw, sem_i.at[NX + NT + 1])
    wg_copy = pltpu.make_async_copy(wg_hbm, wg_v, sem_i.at[NX + NT + 2])
    wu_copy = pltpu.make_async_copy(wu_hbm, wu_v, sem_i.at[NX + NT + 3])
    wd_copy = pltpu.make_async_copy(wd_hbm, wd_v, sem_i.at[NX + NT + 4])

    def o_copy(j):
        at = pl.ds(*out_parts[j])
        return pltpu.make_async_copy(out_v.at[at], out_hbm.at[at], sem_o.at[j])

    for cp in (wr_copy, x_copy(0), *[w_copy(c) for c in range(NT - 1)], x_copy(1), w_copy(NT - 1),
               *[x_copy(j) for j in range(2, NX)], wo_copy, wg_copy, wu_copy, wd_copy):
        cp.start()

    lane = lax.broadcasted_iota(I32, (8, 128), 1)
    sub = lax.broadcasted_iota(I32, (8, 128), 0)

    def permute_w(c):
        quad = lane >> 2
        src_tile = [(5 * (((quad - e) * 13) & 31) + e) >> 5 for e in range(NT)]
        src_lane = [(20 * (lane & 31) + 4 * e + (lane >> 5)) & 127 for e in range(NT)]
        for p in range(3):
            for r0 in range(0, 128, 64):
                a = {r: [pltpu.bitcast(wraw[c, pl.ds(r, 16), pl.ds(p * D + t * 128, 128)], I32) for t in range(NT)]
                     for r in range(r0, r0 + 64, 16)}
                for e in range(NT):
                    for r in a:
                        u = a[r][0]
                        for t in range(1, NT):
                            u = jnp.where(src_tile[e] == t, a[r][t], u)
                        wp[pl.ds(c * 64 + r // 2, 8), pl.ds(p * D + e * 128, 128)] = jnp.take_along_axis(
                            u, src_lane[e], axis=1)

    def permute_wo(t):
        cols = pl.ds(t * 128, 128)
        wo_cols[t, pl.ds(0, D // 2), :] = pltpu.bitcast(wo_raw[:, cols], I32)
        for dp in range(DH // 2):
            ev = wo_cols[t, pl.ds(dp, H // 2, stride=DH), :]
            od = wo_cols[t, pl.ds(dp + DH // 2, H // 2, stride=DH), :]
            wop[pl.ds(dp * H, H // 2), cols] = (ev & 0xFFFF) | (od << 16)
            wop[pl.ds(dp * H + H // 2, H // 2), cols] = lax.shift_right_logical(ev, 16) | (od & -65536)

    score = [jnp.zeros((8, 128), F32) for _ in range(S // 1024)]

    def layernorm(j):
        def rows(g):
            mean = jnp.sum(x_v[pl.ds(g * 16, 16), :].astype(F32), axis=-1, keepdims=True) * (1.0 / D)
            yield
            mb = _rb(mean)
            c = x_v[pl.ds(g * 16, 16), :].astype(F32) - mb
            dm = mean - mb
            var = jnp.sum(c * c, axis=-1, keepdims=True)
            yield
            var = jnp.maximum(var * (1.0 / D) - dm * dm, 0.0)
            den = _rb(jnp.sqrt(_rb(_rb(var) + _rb(jnp.full_like(var, 1e-5)))))
            xn = c * pltpu.reciprocal(den, approx=True)
            xn_v[pl.ds(g * 8, 8), :] = pltpu.bitcast(xn.astype(BF16), I32)
            wrow = wrb[...]
            rr = [jnp.sum(xn[hf * 8:(hf + 1) * 8] * wrow, axis=-1, keepdims=True) for hf in range(2)]
            yield
            for hf in range(2):
                i = 2 * g + hf
                score[i // 128] = jnp.where(lane == (i % 128), rr[hf], score[i // 128])

        r0, n = x_parts[j]
        return _pipeline(range(r0 // 16, (r0 + n) // 16), rows), n // 16 + 3

    def qkv_dst(b):
        qd, kd, vd = bufs[b & 1]
        return [(ref, e, off) for ref, off in ((qd, 0), (kd, HALO), (vd, HALO)) for e in range(NT)]

    def qkv_first(c):
        n = blocks[0][1]
        res = jnp.dot(_bf16(xn_v[pl.ds(0, n // 2), pl.ds(c * 128, 128)]), _bf16(wp[pl.ds(c * 64, 64), :]),
                      preferred_element_type=F32)
        for j, (ref, e, off) in enumerate(qkv_dst(0)):
            part = res[:, j * 128:(j + 1) * 128]
            if c > 0:
                part = part + ref[e, pl.ds(off, n), :]
            ref[e, pl.ds(off, n), :] = part

    def qkv(b):
        r0, n = blocks[b]
        res = jnp.dot(_bf16(xn_v[pl.ds(r0 // 2, n // 2), :]), _bf16(wp[...]), preferred_element_type=F32)
        for j, (ref, e, off) in enumerate(qkv_dst(b)):
            ref[e, pl.ds(off, n), :] = res[:, j * 128:(j + 1) * 128]

    def qkv_pieces(b):
        r0, n = blocks[b]
        m = n // 2

        def gen():
            for j, (ref, e, off) in enumerate(qkv_dst(b)):
                for r in (0, m):
                    ref[e, pl.ds(off + r, m), :] = jnp.dot(
                        _bf16(xn_v[pl.ds((r0 + r) // 2, m // 2), :]), _bf16(wp[:, pl.ds(j * 128, 128)]),
                        preferred_element_type=F32)
                    yield

        return gen(), 6 * NT

    def halo(b):
        for i in (1, 2):
            for e in range(NT):
                bufs[b & 1][i][e, pl.ds(0, HALO), :] = bufs[1 - (b & 1)][i][e, pl.ds(blocks[b - 1][1], HALO), :]

    def attention(b):
        q_v, k_v, v_v = bufs[b & 1]
        r0, n = blocks[b]
        held = {}

        def rows(r):
            q = [q_v[e, pl.ds(r, 8), :] * (scale * LOG2E) for e in range(NT)]
            ls = []
            for w in range(W):
                a = None
                for e in range(NT):
                    t = q[e] * k_v[e, pl.ds(HALO + r - DIL * w, 8), :]
                    a = t if a is None else a + t
                ls.append(a)
            rs = [pltpu.roll(a, 64, 1) for a in ls]
            yield
            ls = [a + c for a, c in zip(ls, rs)]
            rs = [pltpu.roll(a, 32, 1) for a in ls]
            yield
            ls = [a + c for a, c in zip(ls, rs)]
            for w in range(W):
                if r0 + r - DIL * w < 0:
                    ls[w] = jnp.where(sub + (r0 + r - DIL * w) >= 0, ls[w], -1e9 * LOG2E)
            m = functools.reduce(jnp.maximum, ls)
            ps = [jnp.exp2(l - m) for l in ls]
            inv = pltpu.reciprocal(functools.reduce(jnp.add, ps), approx=True)
            o = []
            for e in range(NT):
                a = None
                for w in range(W):
                    t = ps[w] * v_v[e, pl.ds(HALO + r - DIL * w, 8), :]
                    a = t if a is None else a + t
                o.append(a * inv)
            if r % 16 == 0:
                held[r] = o
                return
            prev = held.pop(r - 8)
            for e in range(NT):
                o_v[pl.ds((r0 + r - 8) // 2, 8), pl.ds(e * 128, 128)] = pltpu.bitcast(
                    jnp.concatenate([prev[e], o[e]], axis=0).astype(BF16), I32)

        return _pipeline(range(0, n, 8), rows), n // 8 + 2

    row16 = lax.broadcasted_iota(I32, (16, D), 0)

    def tile_of(i):
        return pl.ds(pl.multiple_of((i >> 4) << 3, 8), 8)

    def route(res):
        rs = [_rb(a) for a in score]
        toks = [((j * 128 + lane) * 8 + sub).astype(F32) for j in range(len(rs))]

        def top(rs):
            m = functools.reduce(jnp.maximum, rs)
            mx = jnp.max(jnp.max(m, axis=1, keepdims=True), axis=0, keepdims=True)
            c = functools.reduce(jnp.minimum, [jnp.where(a == mx, t, float(S)) for a, t in zip(rs, toks)])
            return mx, jnp.min(jnp.min(c, axis=1, keepdims=True), axis=0, keepdims=True)

        m0, i0 = top(rs)
        m1, i1 = top([jnp.where(t == i0, -jnp.inf, a) for a, t in zip(rs, toks)])
        idx = [jnp.clip(i.astype(I32)[0, 0], 0, S - 1) for i in (i0, i1)]
        sel = [jnp.sum(jnp.where(row16 == (i & 15), _bf16(xn_v[tile_of(i), :]).astype(F32), 0.0),
                       axis=0, keepdims=True) for i in idx]
        xs = jnp.where(row16 == 0, sel[0], jnp.where(row16 == 1, sel[1], 0.0)).astype(BF16)
        res.extend((xs, idx, (m0, m1)))
        yield

    def ffn_in(xs, res):
        for n0 in range(0, FF, 128):
            at = pl.ds(n0, min(128, FF - n0))
            g = _rb(lax.dot_general(xs, wg_v[at, :], NT_DIMS, preferred_element_type=F32))
            yield
            u = _rb(lax.dot_general(xs, wu_v[at, :], NT_DIMS, preferred_element_type=F32))
            res.append((g, u))
            yield

    def ffn_out(hid, res):
        acc = None
        for j, n0 in enumerate(range(0, FF, 128)):
            t = jnp.dot(hid[j], wd_v[pl.ds(n0, min(128, FF - n0)), :], preferred_element_type=F32)
            acc = t if acc is None else acc + t
            yield
        res.append(_rb(acc))

    def ffn_apply(y, idx, ms):
        for j, m in enumerate(ms):
            yj = _rb(y[j:j + 1, :] * _rb(1.0 / (1.0 + jnp.exp(-m))))
            tile = _bf16(xn_v[tile_of(idx[j]), :]).astype(F32)
            tile = jnp.where(row16 == (idx[j] & 15), tile + yj, tile)
            xn_v[tile_of(idx[j]), :] = pltpu.bitcast(tile.astype(BF16), I32)

    def out_proj(j):
        r0, n = out_parts[j]
        s = jnp.dot(_bf16(o_v[pl.ds(r0 // 2, n // 2), :]), _bf16(wop[...]), preferred_element_type=F32)
        for e in range(NT):
            cols = pl.ds(e * 128, 128)
            for r in range(0, n, 32):
                z = _bf16(xn_v[pl.ds((r0 + r) // 2, 16), cols]).astype(F32)
                out_v[pl.ds(r0 + r, 32), cols] = (
                    x_v[pl.ds(r0 + r, 32), cols].astype(F32)
                    + s[r:r + 32, e * 128:(e + 1) * 128] * _silu(z)).astype(BF16)
                yield
        o_copy(j).start()

    wr_copy.wait()
    wrb[...] = jnp.broadcast_to(wr_v[...].astype(F32).reshape(1, D), (8, D))
    x_copy(0).wait()
    _run(layernorm(0)[0])
    w_copy(0).wait()
    permute_w(0)
    for c in range(NT):
        if c + 1 < NT:
            w_copy(c + 1).wait()
        if c >= NT - 2:
            x_copy(c - NT + 3).wait()
        qkv_first(c)
        if c + 1 < NT:
            permute_w(c + 1)
        if c >= NT - 2:
            _run(layernorm(c - NT + 3)[0])
        if c == NT - 1:
            for e in range(NT):
                k0[e, pl.ds(0, HALO), :] = jnp.zeros((HALO, 128), F32)
                v0[e, pl.ds(0, HALO), :] = jnp.broadcast_to(v0[e, pl.ds(HALO, 1), :], (HALO, 128))

    x_copy(3).wait()
    halo(1)
    qkv(1)
    _mix(attention(0), layernorm(3))

    routed, gu, y = [], [], []
    x_copy(4).wait()
    halo(2)
    qkv(2)
    ln, n_ln = layernorm(4)
    _mix(attention(1), (_chain(ln, route(routed)), 1.4 * n_ln))
    xs, idx, ms = routed

    wo_copy.wait()
    wg_copy.wait()
    wu_copy.wait()
    halo(3)
    _mix(qkv_pieces(3), (ffn_in(xs, gu), 2 * NF + 2))
    _run(attention(2)[0])
    for t in range(2):
        permute_wo(t)

    wd_copy.wait()
    halo(4)
    hid = [(_rb(_silu(g)) * u).astype(BF16) for g, u in gu]
    _mix(qkv_pieces(4), (ffn_out(hid, y), NF + 1))
    _run(attention(3)[0])
    for t in range(2, NT):
        permute_wo(t)

    pl.semaphore_signal(sem_f, 1)
    pl.semaphore_wait(sem_f, 1)
    ffn_apply(y[0], idx, ms)
    early = sum(r0 + n <= blocks[-1][0] for r0, n in out_parts)
    _mix(attention(4), (_chain(*[out_proj(j) for j in range(early)]), out_parts[early][0] * NT // 32))
    _run(_chain(*[out_proj(j) for j in range(early, len(out_parts))]))
    for j in range(len(out_parts)):
        o_copy(j).wait()


@jax.jit
def pallas_recurrent_scan__sliding_local_dilated__moe_arch_mod__prompt_kernel(
        A_x, A_wqkv, A_wo, B_x, B_w_r, B_w_gate, B_w_up, B_w_down):
    del B_x
    Bn, S, D = A_x.shape
    assert (Bn, S, D) == (1, sum(QKV_BLOCKS), 640)
    Fd = B_w_gate.shape[1]
    NT = D // 128
    T = max(QKV_BLOCKS)
    hbm = pl.BlockSpec(memory_space=pltpu.HBM)
    qkv_bufs = [
        pltpu.VMEM((NT, T, 128), F32),
        pltpu.VMEM((NT, T + HALO, 128), F32),
        pltpu.VMEM((NT, T + HALO, 128), F32),
    ]
    out = pl.pallas_call(
        _kernel,
        in_specs=[hbm] * 7,
        out_specs=hbm,
        out_shape=jax.ShapeDtypeStruct((S, D), A_x.dtype),
        scratch_shapes=[
            pltpu.VMEM((S, D), BF16),
            pltpu.VMEM((NT, 128, 3 * D), BF16),
            pltpu.VMEM((D // 2, 3 * D), I32),
            pltpu.VMEM((D, D), BF16),
            pltpu.VMEM((NT, D // 2 + 24, 128), I32),
            pltpu.VMEM((D // 2, D), I32),
            pltpu.VMEM((D,), BF16),
            pltpu.VMEM((8, D), F32),
            pltpu.VMEM((Fd, D), BF16),
            pltpu.VMEM((Fd, D), BF16),
            pltpu.VMEM((Fd, D), BF16),
            pltpu.VMEM((S // 2, D), I32),
            *qkv_bufs, *qkv_bufs,
            pltpu.VMEM((S // 2, D), I32),
            pltpu.VMEM((S, D), BF16),
            pltpu.SemaphoreType.DMA((len(LN_PARTS) + NT + 5,)),
            pltpu.SemaphoreType.DMA((len(OUT_PARTS),)),
            pltpu.SemaphoreType.REGULAR,
        ],
        compiler_params=pltpu.CompilerParams(
            vmem_limit_bytes=64 * 2**20,
            flags={"XLA_TPU_EVENLY_DISTRIBUTE_CRITICAL_NODES": True}),
    )(A_x.reshape(S, D), A_wqkv, A_wo, B_w_r, B_w_gate.T, B_w_up.T, B_w_down)
    return out.reshape(Bn, S, D)
```
